```python
import os as _os
_os.environ.setdefault('JAX_PLATFORMS', 'cpu')
import jax
import jax.numpy as jnp

def _softmax(x, axis=-1):
    return jax.nn.softmax(x, axis=axis)

def _gelu(x):
    return jax.nn.gelu(x, approximate=True)

def _silu(x):
    return jax.nn.silu(x)

def _sigmoid(x):
    return jax.nn.sigmoid(x)

def _layernorm(x, axis=-1, eps=1e-05):
    m = jnp.mean(x, axis=axis, keepdims=True)
    v = jnp.var(x, axis=axis, keepdims=True)
    return (x - m) / jnp.sqrt(v + eps)

def _scatter_add(tgt, idx, src, axis=0):
    return tgt.at[idx].add(src)

def _segment_sum(src, seg, n):
    return jax.ops.segment_sum(src, seg, n)

class _Rng:

    def __init__(self, key):
        self._k = key

    def _next(self):
        self._k, sub = jax.random.split(self._k)
        return sub

    def normal(self, shape):
        return jax.random.normal(self._next(), shape, dtype=jnp.bfloat16)

    def randint(self, lo, hi, shape):
        return jax.random.randint(self._next(), shape, lo, hi, dtype=jnp.int32)

    def uniform(self, shape, lo=0.0, hi=1.0):
        return jax.random.uniform(self._next(), shape, jnp.bfloat16, lo, hi)

    def permutation(self, n):
        return jax.random.permutation(self._next(), n)
kernel_name = 'parallel_sum__memory_aug_recurrent_mem_tr__dense_activation_silu__prompt'

def setup_inputs():
    _rng = _Rng(jax.random.key(int.from_bytes(__import__("os").urandom(4), "little")))
    _w = lambda a: (lambda t: t.astype(jnp.bfloat16) if jnp.issubdtype(t.dtype, jnp.floating) else t)(jnp.asarray(a))

    def _A_setup():
        B, S, Dm = (1, 2048, 448)
        H, Dh = (16, 256)
        M, seg = (8, 32)
        seg = min(seg, S)
        S = S // seg * seg
        return {'x': _w((lambda *s: _rng.normal(s) * 0.05)(B, S, Dm)), 'mem0': _w((lambda *s: _rng.normal(s) * 0.2)(B, M, Dm)), 'Wq': _w((lambda *s: _rng.normal(s) * 0.8)(Dm, H, Dh) * Dm ** (-0.5)), 'Wk': _w((lambda *s: _rng.normal(s) * 0.8)(Dm, H, Dh) * Dm ** (-0.5)), 'Wv': _w((lambda *s: _rng.normal(s) * 0.2)(Dm, H, Dh) * Dm ** (-0.5)), 'Wo': _w((lambda *s: _rng.normal(s) * 0.2)(H, Dh, Dm) * (H * Dh) ** (-0.5)), 'seg_len': seg}
    _A_in = _A_setup()

    def _B_setup():
        B, S, D, F = (1, 2048, 448, 1792)
        return {'x': _w((lambda *s: _rng.normal(s) * 0.05)(B, S, D)), 'w1': _w((lambda *s: _rng.normal(s) * 0.05)(D, F) * D ** (-0.5)), 'w2': _w((lambda *s: _rng.normal(s) * 0.05)(F, D) * F ** (-0.5))}
    _B_in = _B_setup()
    return {'A_x': _A_in['x'], 'A_mem0': _A_in['mem0'], 'A_Wq': _A_in['Wq'], 'A_Wk': _A_in['Wk'], 'A_Wv': _A_in['Wv'], 'A_Wo': _A_in['Wo'], 'A_seg_len': _A_in['seg_len'], 'B_x': _B_in['x'], 'B_w1': _B_in['w1'], 'B_w2': _B_in['w2']}

def reference(A_x, A_mem0, A_Wq, A_Wk, A_Wv, A_Wo, A_seg_len, B_x, B_w1, B_w2):

    def _A_ref(x, mem0, Wq, Wk, Wv, Wo, seg_len):
        B, S, Dm = x.shape
        H, Dh = (Wq.shape[1], Wq.shape[2])
        M = mem0.shape[1]
        scale = Dh ** (-0.5)
        n_seg = S // seg_len
        L = M + seg_len
        idx = jnp.arange(L)
        mask = (idx[:, None] < M) | (idx[:, None] >= idx[None, :])
        mem = mem0
        outs = []
        for s in range(n_seg):
            xs = x[:, s * seg_len:(s + 1) * seg_len, :].copy()
            h = jnp.concatenate([mem, xs], axis=1)
            q = jnp.einsum('btd,dhe->bhte', h, Wq)
            k = jnp.einsum('btd,dhe->bhte', h, Wk)
            v = jnp.einsum('btd,dhe->bhte', h, Wv)
            scores = jnp.einsum('bhqe,bhke->bhqk', q, k) * scale
            scores = jnp.where(mask[None, None], scores, -1000000000.0)
            p = _softmax(scores, axis=-1)
            o = jnp.einsum('bhqk,bhke->bhqe', p, v)
            o = jnp.einsum('bhte,hed->btd', o, Wo)
            mem = o[:, :M, :].copy()
            outs.append(o[:, M:, :])
        return jnp.concatenate(outs, axis=1)

    def _B_ref(x, w1, w2):
        h = jnp.einsum('bsd,df->bsf', x, w1)
        h = _silu(h)
        out = jnp.einsum('bsf,fd->bsd', h, w2)
        return out
    x = A_x
    xn = _layernorm(x, axis=-1)
    return x + _A_ref(xn, A_mem0, A_Wq, A_Wk, A_Wv, A_Wo, A_seg_len) + _B_ref(xn, B_w1, B_w2)
```

```python
import jax
import jax.numpy as jnp
import numpy as np
from jax import lax
import jax.experimental.pallas as pl
import jax.experimental.pallas.tpu as pltpu

S, D, H, DH, M, SEG, F = 2048, 448, 16, 256, 8, 32, 1792
NPAIR = S // (2 * SEG)
BF, F32, U32 = jnp.bfloat16, jnp.float32, jnp.uint32
EXP2_SCALE = float(DH ** -0.5 * np.log2(np.e))
LOG2E = float(np.log2(np.e))
FILL = -1e9 * DH ** 0.5
NT = (((1,), (1,)), ((), ()))
W2H = 10
TB = 256
NB = S // TB
GD = 64
NG = D // GD


def _caps():
    def keys(c):
        seg = (c >= 40).astype(jnp.int32)
        mem = ((c >= 32) & (c < 40)) | ((c >= 64) & (c < 72))
        idx = jnp.where(c < 32, c, jnp.where(c < 64, c - 40, c - 48))
        return seg, mem, idx
    def cap(qseg, qmem, qidx, c):
        kseg, kmem, kidx = keys(c)
        vis = (qseg == kseg) & (qmem | kmem | (kidx <= qidx))
        return jnp.where(vis, jnp.float32(3e38), jnp.float32(FILL))
    r = lax.broadcasted_iota(jnp.int32, (32, 48), 0)
    c = lax.broadcasted_iota(jnp.int32, (32, 48), 1)
    ce = cap(jnp.zeros_like(r), r < 8, r - 8, c)
    r = lax.broadcasted_iota(jnp.int32, (48, 80), 0)
    c = lax.broadcasted_iota(jnp.int32, (48, 80), 1)
    qseg = 1 - ((r >= 32) & (r < 40)).astype(jnp.int32)
    qidx = jnp.where(r < 16, r + 16, jnp.where(r < 32, r - 8, jnp.where(r < 40, r - 8, r - 40)))
    co = cap(qseg, r < 8, qidx, c)
    return ce, co


def _softmax_p(s, cap):
    s = jnp.minimum(s, cap)
    m = jnp.max(s, axis=-1, keepdims=True)
    e = jnp.exp2((s - m) * EXP2_SCALE)
    l = jnp.sum(e, axis=-1, keepdims=True)
    return (e * pl.reciprocal(l, approx=True)).astype(BF)


def _bf(ref_u32, idx=...):
    return pltpu.bitcast(ref_u32[idx], BF)


def _kernel(xT_hbm, mem0_hbm, wq_hbm, wk_hbm, wv_hbm, woT_hbm, w1_hbm, w2T_hbm,
            outT_hbm,
            xT_ref, mem0_ref, wst_ref, woT_ref, w1_ref, w2T_ref, outT_ref,
            xn_ref, w_ref, wo_ref, w2u_ref, orow_ref, act_ref,
            kg_ref, vg_ref, q8a_ref, q16_ref, q8b_ref, ce_ref, co_ref,
            sems, wsems, osem):
    cp_x0 = pltpu.make_async_copy(xT_hbm.at[:, 0:TB], xT_ref.at[:, 0:TB], sems.at[0])
    cp_w1 = pltpu.make_async_copy(w1_hbm, w1_ref, sems.at[1])
    cp_x1 = pltpu.make_async_copy(xT_hbm.at[:, TB:S], xT_ref.at[:, TB:S], sems.at[2])
    cp_m = pltpu.make_async_copy(mem0_hbm, mem0_ref, sems.at[3])
    cp_wo = pltpu.make_async_copy(woT_hbm, woT_ref, sems.at[4])
    cp_w2 = pltpu.make_async_copy(w2T_hbm, w2T_ref, sems.at[5])

    def cp_w(g, mi):
        src = (wq_hbm, wk_hbm, wv_hbm)[mi // 2]
        c = mi % 2
        r0 = g * GD * H if isinstance(g, int) else pl.multiple_of(g * GD * H, GD * H)
        return pltpu.make_async_copy(src.at[pl.ds(r0, GD * H), c * 128:(c + 1) * 128],
                                     wst_ref.at[mi, pl.ds(r0, GD * H)], wsems.at[g])

    cp_x0.start()
    cp_w1.start()
    cp_x1.start()
    cp_m.start()

    ce, co = _caps()
    ce_ref[...] = ce
    co_ref[...] = co
    orow_ref[0:128, :] = jnp.zeros((128, D), F32)

    def ln(t0):
        x = xT_ref[:, pl.ds(t0, 128)].astype(F32)
        mu = jnp.mean(x, axis=0, keepdims=True)
        xc = x - mu
        var = jnp.mean(xc * xc, axis=0, keepdims=True)
        xn_ref[pl.ds(t0, 128), :] = (xc / jnp.sqrt(var + 1e-5)).T

    wst_u = wst_ref.bitcast(U32)

    def relayout_unit(g, cc, mi):
        d0 = g * GD + cc * 16
        r0 = g * (GD // 2) + cc * 8
        row = d0 * 8
        if not isinstance(g, int):
            row = pl.multiple_of(row, 128)
            r0 = pl.multiple_of(r0, 8)
        for c in range(2):
            win = wst_u.at[2 * mi + c, pl.ds(row, 128)]
            for j in range(H // 2):
                ev = win[pl.ds(j, 8, stride=16), :]
                od = win[pl.ds(8 + j, 8, stride=16), :]
                col = 2 * j * 768 + mi * 256 + c * 128
                w_ref[pl.ds(r0, 8), col:col + 128] = (ev & jnp.uint32(0xFFFF)) | (od << 16)
                w_ref[pl.ds(r0, 8), col + 768:col + 896] = (ev >> 16) | (od & jnp.uint32(0xFFFF0000))

    def pro_block(b, do_ln, g):
        t0 = b * TB if isinstance(b, int) else pl.multiple_of(b * TB, TB)
        side = []
        if do_ln:
            for u in range(TB // 128):
                t1 = (b + 1) * TB + u * 128
                side.append(("ln", t1 if isinstance(b, int) else pl.multiple_of(t1, 128)))
        if g is not None:
            side += [("rl", cc, mi) for cc in range(GD // 16) for mi in range(3)]
        MB = 128
        nsub = TB // MB
        done = 0
        for c in range(nsub):
            ts = t0 + c * MB
            if not isinstance(b, int):
                ts = pl.multiple_of(ts, MB)
            xb = xn_ref[pl.ds(ts, MB), :].astype(BF)
            hf = jnp.dot(xb, w1_ref[...], preferred_element_type=F32)
            e_ = jnp.exp2(hf * (-LOG2E))
            act_ref[pl.ds(ts, MB), :] = (hf * pl.reciprocal(1.0 + e_, approx=True)).astype(BF)
            upto = (c + 1) * len(side) // nsub
            for s_ in side[done:upto]:
                if s_[0] == "ln":
                    ln(s_[1])
                else:
                    relayout_unit(g, s_[1], s_[2])
            done = upto

    LA = 3
    cp_x0.wait()
    ln(0)
    ln(128)
    cp_w1.wait()
    for g in range(LA):
        for mi in range(6):
            cp_w(g, mi).start()
    cp_x1.wait()
    pro_block(0, True, None)
    for mi in range(6):
        cp_w(0, mi).wait()

    def pro_body(b, c):
        @pl.when(b - 1 + LA < NG)
        def _():
            for mi in range(6):
                cp_w(b - 1 + LA, mi).start()
        @pl.when(b - 1 + LA == NG)
        def _():
            cp_wo.start()
            cp_w2.start()
        pro_block(b, True, b - 1)
        for mi in range(6):
            cp_w(b, mi).wait()
        return c
    lax.fori_loop(1, NB - 1, pro_body, 0)
    pro_block(NB - 1, False, NG - 1)

    def store_next(Rh, h, r0):
        hs = slice(h * 256, (h + 1) * 256)
        q8a_ref[:, hs] = Rh[r0:r0 + 8, 0:256]
        q16_ref[:, hs] = Rh[r0 + 8:r0 + 24, 0:256].astype(BF)
        q8b_ref[:, hs] = Rh[r0 + 24:r0 + 32, 0:256]
        kg_ref[:, hs] = Rh[r0:r0 + 32, 256:512].astype(BF)
        vg_ref[:, hs] = Rh[r0:r0 + 32, 512:768].astype(BF)

    def wcols(h, z):
        return _bf(w_ref, (pl.ds(z, D // 2), slice(h * 768, (h + 1) * 768)))

    lhs0 = xn_ref[0:32, :].astype(BF)
    cp_wo.wait()
    for h in range(H):
        store_next(jnp.dot(lhs0, wcols(h, 0), preferred_element_type=F32), h, 0)
        wo_ref[h * 128:(h + 1) * 128, :] = pltpu.bitcast(woT_ref[h].T, U32)
        if h == W2H:
            cp_w2.wait()
        if h >= W2H:
            n_ = H - W2H
            for j in range((h - W2H) * 14 // n_, (h - W2H + 1) * 14 // n_):
                w2u_ref[j * 64:(j + 1) * 64, :] = pltpu.bitcast(w2T_ref[:, j * 128:(j + 1) * 128].T, U32)
    cp_m.wait()

    def out_block(t0):
        y = orow_ref[pl.ds(t0, 128), :].T
        outT_ref[:, pl.ds(t0, 128)] = (xT_ref[:, pl.ds(t0, 128)].astype(F32) + y).astype(BF)

    def cp_out(t0):
        return pltpu.make_async_copy(outT_ref.at[:, pl.ds(t0, 128)], outT_hbm.at[:, pl.ds(t0, 128)], osem)

    def pair(p, mem, sub):
        base = pl.multiple_of(p * 64, 64)
        nxt = pl.multiple_of(jnp.minimum(base + 64, S - 32), 32)
        z = [pl.multiple_of(lax.shift_right_logical(p, 10 + i + 2 * sub) * 8, 8) for i in range(2)]
        cap = (ce_ref[...], co_ref[...])
        V = dict(mem0=mem)
        R = [[None] * H, [None] * H]
        Sc = [[None] * H, [None] * H]
        P = [[None] * H, [None] * H]
        O = [[None] * H, [None] * H]
        KV = [[None] * H, [None] * H]
        C = [None, None]
        FF = []

        def lhs(e):
            if e == 0:
                V['lhs0'] = jnp.concatenate([V['mem0'], xn_ref[pl.ds(base + 32, 24), :]], axis=0).astype(BF)
            else:
                V['lhs1'] = jnp.concatenate([C[0][0:8], xn_ref[pl.ds(base + 56, 8), :], xn_ref[pl.ds(nxt, 32), :]], axis=0).astype(BF)

        def A(e, h):
            R[e][h] = jnp.dot(V['lhs%d' % e], wcols(h, z[e]), preferred_element_type=F32)

        def QK(e, h):
            hs = slice(h * 256, (h + 1) * 256)
            Rh = R[e][h]
            if e == 0:
                gb = Rh[16:32, :].astype(BF)
                gkv = Rh[0:16, 256:768].astype(BF)
                q = jnp.concatenate([
                    jnp.concatenate([Rh[0:8, 0:256], q8a_ref[:, hs]], axis=0).astype(BF),
                    q16_ref[:, hs]], axis=0)
                k = jnp.concatenate([kg_ref[:, hs], gkv[:, 0:256]], axis=0)
                KV[0][h] = (Rh[8:16, 0:256], gkv, gb)
            else:
                gc = Rh[0:16, :].astype(BF)
                qa, gkv, gb = KV[0][h]
                q = jnp.concatenate([
                    gc[:, 0:256], gb[:, 0:256],
                    jnp.concatenate([q8b_ref[:, hs], qa], axis=0).astype(BF)], axis=0)
                k = jnp.concatenate([kg_ref[:, hs], gkv[:, 0:256], gb[:, 256:512], gc[:, 256:512]], axis=0)
                KV[1][h] = gc
            Sc[e][h] = lax.dot_general(q, k, NT, preferred_element_type=F32)

        def SM(e, h):
            P[e][h] = _softmax_p(Sc[e][h], cap[e])

        def PV(e, h):
            hs = slice(h * 256, (h + 1) * 256)
            qa, gkv, gb = KV[0][h]
            if e == 0:
                v = jnp.concatenate([vg_ref[:, hs], gkv[:, 256:512]], axis=0)
            else:
                v = jnp.concatenate([vg_ref[:, hs], gkv[:, 256:512], gb[:, 512:768], KV[1][h][:, 512:768]], axis=0)
            O[e][h] = jnp.dot(P[e][h], v, preferred_element_type=F32).astype(BF)

        def ST(h):
            store_next(R[1][h], h, 16)

        def Call(e):
            o = jnp.concatenate(O[e], axis=1)
            C[e] = jnp.dot(o, _bf(wo_ref, (pl.ds(z[e], 2048), slice(None))), preferred_element_type=F32)

        def Ch(e, h0, h1):
            o = jnp.concatenate(O[e][h0:h1], axis=1) if h1 - h0 > 1 else O[e][h0]
            t = jnp.dot(o, _bf(wo_ref, (pl.ds(z[e] + h0 * 128, (h1 - h0) * 128), slice(None))), preferred_element_type=F32)
            C[e] = t if C[e] is None else C[e] + t

        def F1(j0, j1):
            pass

        def F2(j0, j1):
            a = act_ref[pl.ds(base, 64), j0 * 128:j1 * 128]
            FF.append(jnp.dot(a, _bf(w2u_ref, (slice(j0 * 64, j1 * 64), slice(None))), preferred_element_type=F32))

        lhs(0)
        for h in range(H): A(0, h)
        for h in range(H): QK(0, h)
        F2(0, 4)
        for h in range(H): SM(0, h); PV(0, h)
        Call(0)
        F2(4, 7)
        lhs(1)
        for h in range(H): A(1, h)
        for h in range(H): QK(1, h)
        F2(7, 11)
        for h in range(H): SM(1, h); PV(1, h); ST(h)
        Call(1)
        F2(11, 14)
        Ce, Co = C
        tot = jnp.concatenate([Ce[8:32], Co[32:40], Co[40:48], Co[16:32], Co[8:16]], axis=0)
        for f_ in FF:
            tot = tot + f_
        orow_ref[pl.ds(base, 64), :] = tot
        return Co[0:8]

    def body(i, mem):
        tprev = pl.multiple_of(jnp.maximum(i - 1, 0) * 128, 128)
        out_block(tprev)
        @pl.when(i > 0)
        def _():
            cp_out(tprev).start()
        for u in range(2):
            mem = pair(i * 2 + u, mem, u)
        return mem
    lax.fori_loop(0, NPAIR // 2, body, mem0_ref[...].astype(F32))

    out_block(S - 128)
    cp_out(S - 128).start()
    for b in list(range(NPAIR // 2 - 1)) + [S // 128 - 1]:
        cp_out(b * 128).wait()


@jax.jit
def pallas_parallel_sum__memory_aug_recurrent_mem_tr__dense_activation_silu__prompt_kernel(
    A_x, A_mem0, A_Wq, A_Wk, A_Wv, A_Wo, A_seg_len, B_x, B_w1, B_w2):
    x, mem0, wq, wk, wv, wo, w1, w2 = A_x, A_mem0, A_Wq, A_Wk, A_Wv, A_Wo, B_w1, B_w2
    hbm = pl.BlockSpec(memory_space=pltpu.HBM)
    outT = pl.pallas_call(
        _kernel,
        out_shape=jax.ShapeDtypeStruct((D, S), BF),
        in_specs=[hbm] * 8,
        out_specs=hbm,
        scratch_shapes=[
            pltpu.VMEM((D, S), BF),
            pltpu.VMEM((M, D), BF),
            pltpu.VMEM((6, D * H, 128), BF),
            pltpu.VMEM((H, D, DH), BF),
            pltpu.VMEM((D, F), BF),
            pltpu.VMEM((D, F), BF),
            pltpu.VMEM((D, S), BF),
            pltpu.VMEM((S, D), F32),
            pltpu.VMEM((D // 2, 3 * H * DH), U32),
            pltpu.VMEM((H * DH // 2, D), U32),
            pltpu.VMEM((F // 2, D), U32),
            pltpu.VMEM((S, D), F32),
            pltpu.VMEM((S, F), BF),
            pltpu.VMEM((32, H * DH), BF),
            pltpu.VMEM((32, H * DH), BF),
            pltpu.VMEM((8, H * DH), F32),
            pltpu.VMEM((16, H * DH), BF),
            pltpu.VMEM((8, H * DH), F32),
            pltpu.VMEM((32, 48), F32),
            pltpu.VMEM((48, 80), F32),
            pltpu.SemaphoreType.DMA((6,)),
            pltpu.SemaphoreType.DMA((NG,)),
            pltpu.SemaphoreType.DMA(()),
        ],
        compiler_params=pltpu.CompilerParams(vmem_limit_bytes=110 * 1024 * 1024),
    )(jnp.swapaxes(x, 1, 2).reshape(D, S), mem0.reshape(M, D), wq.reshape(D * H, DH), wk.reshape(D * H, DH), wv.reshape(D * H, DH),
      jnp.swapaxes(wo, 1, 2), w1, w2.T)
    return jnp.swapaxes(outT.reshape(1, D, S), 1, 2)
```

```python
import jax
import jax.numpy as jnp
import numpy as np
from jax import lax
import jax.experimental.pallas as pl
import jax.experimental.pallas.tpu as pltpu

S, D, H, DH, M, SEG, F = 2048, 448, 16, 256, 8, 32, 1792
NPAIR = S // (2 * SEG)
UN = 4
TB = 256
NB = S // TB
MB = 64
GD = 64
NG = D // GD
FH = F // 2
BF, F32, U32 = jnp.bfloat16, jnp.float32, jnp.uint32
LOG2E = float(np.log2(np.e))
EXP2_SCALE = float(DH ** -0.5 * LOG2E)
FILL = -1e9 * DH ** 0.5
NT = (((1,), (1,)), ((), ()))
LO16, HI16 = np.uint32(0x0000FFFF), np.uint32(0xFFFF0000)


def _caps():
    def cap(qseg, qmem, qidx, c):
        kseg = (c >= 40).astype(jnp.int32)
        kmem = ((c >= 32) & (c < 40)) | ((c >= 64) & (c < 72))
        kidx = jnp.where(c < 32, c, jnp.where(c < 64, c - 40, c - 48))
        vis = (qseg == kseg) & (qmem | kmem | (kidx <= qidx))
        return jnp.where(vis, 3e38, FILL).astype(F32)
    r = lax.broadcasted_iota(jnp.int32, (32, 48), 0)
    c = lax.broadcasted_iota(jnp.int32, (32, 48), 1)
    ce = cap(jnp.zeros_like(r), r < 8, r - 8, c)
    r = lax.broadcasted_iota(jnp.int32, (48, 80), 0)
    c = lax.broadcasted_iota(jnp.int32, (48, 80), 1)
    qseg = 1 - ((r >= 32) & (r < 40)).astype(jnp.int32)
    qidx = jnp.where(r < 16, r + 16, jnp.where(r < 40, r - 8, r - 40))
    co = cap(qseg, r < 8, qidx, c)
    return ce, co


def _softmax_p(s, cap):
    s = jnp.minimum(s, cap)
    m = jnp.max(s, axis=-1, keepdims=True)
    e = jnp.exp2((s - m) * EXP2_SCALE)
    l = jnp.sum(e, axis=-1, keepdims=True)
    return (e * pl.reciprocal(l, approx=True)).astype(BF)


def _bf(ref_u32, idx=...):
    return pltpu.bitcast(ref_u32[idx], BF)


def _transpose8(X):
    sub = lax.broadcasted_iota(jnp.int32, (8, 128), 0)
    X = list(X)
    for k in (4, 2, 1):
        m = (sub & k) != 0
        Y = list(X)
        for s in range(8):
            if not s & k:
                Y[s] = jnp.where(m, pltpu.roll(X[s + k], k, 0), X[s])
                Y[s + k] = jnp.where(m, X[s + k], pltpu.roll(X[s], 8 - k, 0))
        X = Y
    return X


def _ds(start, size, align):
    if not isinstance(start, int):
        start = pl.multiple_of(start, align)
    return pl.ds(start, size)


def _kernel(xT_hbm, mem0_hbm, wq_hbm, wk_hbm, wv_hbm, woT_hbm, w1_hbm, w2T_hbm,
            outT_hbm,
            xT_ref, mem0_ref, wst_ref, woT_ref, w1_ref, w2T_ref, outT_ref,
            xn_ref, xnu_ref, w_ref, wo_ref, w1u_ref, w2u_ref, orow_ref, act_ref,
            kg_ref, vg_ref, q8a_ref, q16_ref, q8b_ref, ce_ref, co_ref,
            sems, xsems, wsems, osem):
    def cp_x(b):
        cols = _ds(b * TB, TB, TB)
        return pltpu.make_async_copy(xT_hbm.at[:, cols], xT_ref.at[:, cols], xsems.at[b])

    cp_w1 = [pltpu.make_async_copy(w1_hbm.at[:, i * FH:(i + 1) * FH],
                                   w1_ref.at[:, i * FH:(i + 1) * FH], sems.at[i]) for i in range(2)]
    cp_m = pltpu.make_async_copy(mem0_hbm, mem0_ref, sems.at[2])
    cp_w2 = pltpu.make_async_copy(w2T_hbm, w2T_ref, sems.at[3])

    def cp_wo(i):
        heads = _ds(4 * i, 4, 4)
        return pltpu.make_async_copy(woT_hbm.at[heads], woT_ref.at[heads], sems.at[4 + i])

    def cp_w(g, mi):
        src = (wq_hbm, wk_hbm, wv_hbm)[mi // 2]
        c = mi % 2
        rows = _ds(g * GD * H, GD * H, GD * H)
        return pltpu.make_async_copy(src.at[rows, c * 128:(c + 1) * 128], wst_ref.at[mi, rows], wsems.at[g])

    def start_group(g):
        for mi in range(6):
            cp_w(g, mi).start()

    def wait_group(g):
        for mi in range(6):
            cp_w(g, mi).wait()

    def issue_a(k, c):
        pl.when(k == 0)(cp_x(0).start)
        pl.when(k == 1)(cp_w1[0].start)
        pl.when(k == 2)(cp_w1[1].start)

        @pl.when(k == 3)
        def _():
            cp_x(1).start()
            cp_x(2).start()
            cp_m.start()
        return c
    lax.fori_loop(0, 4, issue_a, 0)

    def issue_w(g, c):
        start_group(g)

        @pl.when(g + 3 < NB)
        def _():
            cp_x(g + 3).start()
        return c
    lax.fori_loop(0, NG, issue_w, 0)

    def issue_wo(i, c):
        pl.when(i == 2)(cp_w2.start)
        cp_wo(i).start()
        return c
    lax.fori_loop(0, 4, issue_wo, 0)

    ce, co = _caps()
    ce_ref[...] = ce
    co_ref[...] = co
    orow_ref[0:128, :] = jnp.zeros((128, D), F32)

    def ln(t0):
        x = xT_ref[:, _ds(t0, 128, 128)].astype(F32)
        mu = jnp.mean(x, axis=0, keepdims=True)
        xc = x - mu
        var = jnp.mean(xc * xc, axis=0, keepdims=True)
        xn = (xc / jnp.sqrt(var + 1e-5)).T
        xn_ref[_ds(t0, 128, 128), :] = xn
        xnu_ref[_ds(t0 // 2, 64, 64), :] = pltpu.bitcast(xn.astype(BF), U32)

    def silu_store(hf, t0, n, c0, c1):
        e = jnp.exp2(hf * (-LOG2E))
        act_ref[_ds(t0, n, n), c0:c1] = (hf * pl.reciprocal(1.0 + e, approx=True)).astype(BF)

    wst_u = wst_ref.bitcast(U32)

    def relayout_unit(g, cc, mi, c, m_lo, m_hi):
        d0 = g * GD + cc * 16
        blk = wst_u[2 * mi + c, _ds(d0 * 8, 128, 128), :]
        V = [blk[8 * d:8 * d + 8] for d in range(16)]
        lo = _transpose8([(V[2 * s] & m_lo) | (V[2 * s + 1] << 16) for s in range(8)])
        hi = _transpose8([(V[2 * s] >> 16) | (V[2 * s + 1] & m_hi) for s in range(8)])
        rows = _ds(g * (GD // 2) + cc * 8, 8, 8)
        for j in range(H // 2):
            col = 2 * j * 768 + mi * 256 + c * 128
            w_ref[rows, col:col + 128] = lo[j]
            w_ref[rows, col + 768:col + 896] = hi[j]

    def wo_unit(h):
        wo_ref[h * 128:(h + 1) * 128, :] = pltpu.bitcast(woT_ref[h].T, U32)

    def w2_unit(j):
        w2u_ref[j * 64:(j + 1) * 64, :] = pltpu.bitcast(w2T_ref[:, j * 128:(j + 1) * 128].T, U32)

    def pro_block(b, do_ln, g, z, extra=()):
        units = [(cc, mi, c) for cc in range(GD // 16) for mi in range(3) for c in range(2)]
        nsub, nslot = TB // MB, (TB // MB) * (F // 128)
        zero_v = jnp.full((8, 128), z, U32)
        k = 0
        for sb in range(nsub):
            ts = b * TB + sb * MB
            xb = _bf(xnu_ref, (_ds(ts // 2, MB // 2, MB // 2), slice(None)))
            hf = jnp.dot(xb, _bf(w1u_ref), preferred_element_type=F32)
            silu_store(hf, ts, MB, 0, F)
            while k < len(units) and (k * nslot) // len(units) < (sb + 1) * (F // 128):
                j = (k * nslot) // len(units) - sb * (F // 128)
                a = pltpu.bitcast(hf[0:8, j * 128:(j + 1) * 128], U32) & zero_v
                relayout_unit(g, *units[k], a | LO16, a | HI16)
                k += 1
            if sb == 0 and do_ln:
                for u in range(TB // 128):
                    ln((b + 1) * TB + u * 128)
            for h in extra[sb * len(extra) // nsub:(sb + 1) * len(extra) // nsub]:
                wo_unit(h)

    cp_x(0).wait()
    ln(0)
    ln(128)
    for i in range(2):
        cp_w1[i].wait()
        if i == 1:
            cp_x(1).wait()
        for u in range(TB // 128):
            xb = _bf(xnu_ref, (pl.ds(u * 64, 64), slice(None)))
            hf = jnp.dot(xb, w1_ref[:, i * FH:(i + 1) * FH], preferred_element_type=F32)
            silu_store(hf, u * 128, 128, i * FH, (i + 1) * FH)
            if i == 1:
                ln(TB + u * 128)
        w1u_ref[:, i * FH:(i + 1) * FH] = pltpu.bitcast(w1_ref[:, i * FH:(i + 1) * FH], U32)

    def pro_body(b, c):
        @pl.when(b + 1 < NB)
        def _():
            cp_x(b + 1).wait()
            wait_group(b - 1)
        z = lax.shift_right_logical(b, 10)
        pro_block(b, True, b - 1, z.astype(U32))
        return z
    z_last = lax.fori_loop(1, NB - 1, pro_body, jnp.int32(0))

    @pl.when(z_last == 0)
    def _():
        wait_group(NG - 1)
        cp_wo(0).wait()
    pro_block(NB - 1, False, NG - 1, z_last.astype(U32), extra=list(range(4)))

    def store_next(Rh, h, r0):
        hs = slice(h * 256, (h + 1) * 256)
        q8a_ref[:, hs] = Rh[r0:r0 + 8, 0:256]
        q16_ref[:, hs] = Rh[r0 + 8:r0 + 24, 0:256].astype(BF)
        q8b_ref[:, hs] = Rh[r0 + 24:r0 + 32, 0:256]
        kg_ref[:, hs] = Rh[r0:r0 + 32, 256:512].astype(BF)
        vg_ref[:, hs] = Rh[r0:r0 + 32, 512:768].astype(BF)

    def wcols(h, z):
        return _bf(w_ref, (pl.ds(z, D // 2), slice(h * 768, (h + 1) * 768)))

    lhs0 = xn_ref[0:32, :].astype(BF)
    WO = lambda a, b: [lambda h=h: wo_unit(h) for h in range(a, b)]
    W2 = lambda a, b: [lambda j=j: w2_unit(j) for j in range(a, b)]
    plan = [([cp_wo(1), cp_w2], WO(4, 8) + W2(0, 7)),
            ([cp_wo(2)], W2(7, 14) + WO(8, 12)),
            ([cp_wo(3), cp_m], WO(12, 16))]
    for part, (waits, side) in enumerate(plan):
        @pl.when(z_last == 0)
        def _():
            for c in waits:
                c.wait()
        done = 0
        for n, h in enumerate(range(8 * part, 8 * part + 8) if part < 2 else ()):
            store_next(jnp.dot(lhs0, wcols(h, 0), preferred_element_type=F32), h, 0)
            upto = (n + 1) * len(side) // 8
            for fn in side[done:upto]:
                fn()
            done = upto
        for fn in side[done:]:
            fn()

    def out_block(t0):
        cols = _ds(t0, 128, 128)
        y = orow_ref[cols, :].T
        outT_ref[:, cols] = (xT_ref[:, cols].astype(F32) + y).astype(BF)

    def cp_out(t0):
        cols = _ds(t0, 128, 128)
        return pltpu.make_async_copy(outT_ref.at[:, cols], outT_hbm.at[:, cols], osem)

    def pair(p, mem, sub):
        base = pl.multiple_of(p * 64, 64)
        nxt = pl.multiple_of(jnp.minimum(base + 64, S - 32), 32)
        z = [pl.multiple_of(lax.shift_right_logical(p, 10 + i + 2 * sub) * 8, 8) for i in range(2)]
        cap = (ce_ref[...], co_ref[...])
        FF = []

        def ffn2(j0, j1):
            a = act_ref[pl.ds(base, 64), j0 * 128:j1 * 128]
            FF.append(jnp.dot(a, _bf(w2u_ref, (slice(j0 * 64, j1 * 64), slice(None))),
                              preferred_element_type=F32))

        def out_proj(o, e):
            return jnp.dot(jnp.concatenate(o, axis=1), _bf(wo_ref, (pl.ds(z[e], H * DH // 2), slice(None))),
                           preferred_element_type=F32)

        lhs = jnp.concatenate([mem, xn_ref[pl.ds(base + 32, 24), :]], axis=0).astype(BF)
        R = [jnp.dot(lhs, wcols(h, z[0]), preferred_element_type=F32) for h in range(H)]
        keep, sc = [], []
        for h in range(H):
            hs = slice(h * 256, (h + 1) * 256)
            gb = R[h][16:32, :].astype(BF)
            gkv = R[h][0:16, 256:768].astype(BF)
            q = jnp.concatenate([
                jnp.concatenate([R[h][0:8, 0:256], q8a_ref[:, hs]], axis=0).astype(BF),
                q16_ref[:, hs]], axis=0)
            k = jnp.concatenate([kg_ref[:, hs], gkv[:, 0:256]], axis=0)
            keep.append((R[h][8:16, 0:256], gkv, gb))
            sc.append(lax.dot_general(q, k, NT, preferred_element_type=F32))
        ffn2(0, 4)
        o = []
        for h in range(H):
            v = jnp.concatenate([vg_ref[:, h * 256:(h + 1) * 256], keep[h][1][:, 256:512]], axis=0)
            o.append(jnp.dot(_softmax_p(sc[h], cap[0]), v, preferred_element_type=F32).astype(BF))
        Ce = out_proj(o, 0)
        ffn2(4, 7)

        lhs = jnp.concatenate([Ce[0:8], xn_ref[pl.ds(base + 56, 8), :], xn_ref[pl.ds(nxt, 32), :]],
                              axis=0).astype(BF)
        R = [jnp.dot(lhs, wcols(h, z[1]), preferred_element_type=F32) for h in range(H)]
        gcs, sc = [], []
        for h in range(H):
            hs = slice(h * 256, (h + 1) * 256)
            qa, gkv, gb = keep[h]
            gc = R[h][0:16, :].astype(BF)
            q = jnp.concatenate([
                gc[:, 0:256], gb[:, 0:256],
                jnp.concatenate([q8b_ref[:, hs], qa], axis=0).astype(BF)], axis=0)
            k = jnp.concatenate([kg_ref[:, hs], gkv[:, 0:256], gb[:, 256:512], gc[:, 256:512]], axis=0)
            gcs.append(gc)
            sc.append(lax.dot_general(q, k, NT, preferred_element_type=F32))
        ffn2(7, 11)
        o = []
        for h in range(H):
            _, gkv, gb = keep[h]
            v = jnp.concatenate([vg_ref[:, h * 256:(h + 1) * 256], gkv[:, 256:512], gb[:, 512:768],
                                 gcs[h][:, 512:768]], axis=0)
            o.append(jnp.dot(_softmax_p(sc[h], cap[1]), v, preferred_element_type=F32).astype(BF))
            store_next(R[h], h, 16)
        Co = out_proj(o, 1)
        ffn2(11, 14)

        tot = jnp.concatenate([Ce[8:32], Co[32:40], Co[40:48], Co[16:32], Co[8:16]], axis=0)
        for f in FF:
            tot = tot + f
        orow_ref[pl.ds(base, 64), :] = tot
        return Co[0:8]

    def body(i, mem):
        for u in range(0, UN, 2):
            tprev = jnp.maximum(i * (UN // 2) + u // 2 - 1, 0) * 128
            out_block(tprev)
            if u == 0:
                @pl.when(i > 0)
                def _():
                    cp_out(tprev).start()
            else:
                cp_out(tprev).start()
            for v in range(2):
                mem = pair(i * UN + u + v, mem, u + v)
        return mem
    lax.fori_loop(0, NPAIR // UN, body, mem0_ref[...].astype(F32))

    out_block(S - 128)
    cp_out(S - 128).start()
    for b in range(S // 128):
        cp_out(b * 128).wait()


@jax.jit
def pallas_parallel_sum__memory_aug_recurrent_mem_tr__dense_activation_silu__prompt_kernel(
    A_x, A_mem0, A_Wq, A_Wk, A_Wv, A_Wo, A_seg_len, B_x, B_w1, B_w2,
):
    hbm = pl.BlockSpec(memory_space=pltpu.HBM)
    outT = pl.pallas_call(
        _kernel,
        out_shape=jax.ShapeDtypeStruct((D, S), BF),
        in_specs=[hbm] * 8,
        out_specs=hbm,
        scratch_shapes=[
            pltpu.VMEM((D, S), BF),
            pltpu.VMEM((M, D), BF),
            pltpu.VMEM((6, D * H, 128), BF),
            pltpu.VMEM((H, D, DH), BF),
            pltpu.VMEM((D, F), BF),
            pltpu.VMEM((D, F), BF),
            pltpu.VMEM((D, S), BF),
            pltpu.VMEM((S, D), F32),
            pltpu.VMEM((S // 2, D), U32),
            pltpu.VMEM((D // 2, 3 * H * DH), U32),
            pltpu.VMEM((H * DH // 2, D), U32),
            pltpu.VMEM((D // 2, F), U32),
            pltpu.VMEM((F // 2, D), U32),
            pltpu.VMEM((S, D), F32),
            pltpu.VMEM((S, F), BF),
            pltpu.VMEM((32, H * DH), BF),
            pltpu.VMEM((32, H * DH), BF),
            pltpu.VMEM((8, H * DH), F32),
            pltpu.VMEM((16, H * DH), BF),
            pltpu.VMEM((8, H * DH), F32),
            pltpu.VMEM((32, 48), F32),
            pltpu.VMEM((48, 80), F32),
            pltpu.SemaphoreType.DMA((8,)),
            pltpu.SemaphoreType.DMA((NB,)),
            pltpu.SemaphoreType.DMA((NG,)),
            pltpu.SemaphoreType.DMA(()),
        ],
        compiler_params=pltpu.CompilerParams(vmem_limit_bytes=110 * 1024 * 1024),
    )(jnp.swapaxes(A_x, 1, 2).reshape(D, S), A_mem0.reshape(M, D),
      A_Wq.reshape(D * H, DH), A_Wk.reshape(D * H, DH), A_Wv.reshape(D * H, DH),
      jnp.swapaxes(A_Wo, 1, 2), B_w1, B_w2.T)
    return jnp.swapaxes(outT.reshape(1, D, S), 1, 2)
```

```python
import jax
import jax.numpy as jnp
import numpy as np
from jax import lax
import jax.experimental.pallas as pl
import jax.experimental.pallas.tpu as pltpu

S, D, H, DH, M, SEG, F = 2048, 448, 16, 256, 8, 32, 1792
NPAIR = S // (2 * SEG)
TB = 256
NB = S // TB
MB = 64
GD = 64
NG = D // GD
FH = F // 2
BF, F32, U32 = jnp.bfloat16, jnp.float32, jnp.uint32
LOG2E = float(np.log2(np.e))
EXP2_SCALE = float(DH ** -0.5 * LOG2E)
FILL = -1e9 * DH ** 0.5
NT = (((1,), (1,)), ((), ()))
LO16, HI16 = np.uint32(0x0000FFFF), np.uint32(0xFFFF0000)


def _caps():
    def cap(qseg, qmem, qidx, c):
        kseg = (c >= 40).astype(jnp.int32)
        kmem = ((c >= 32) & (c < 40)) | ((c >= 64) & (c < 72))
        kidx = jnp.where(c < 32, c, jnp.where(c < 64, c - 40, c - 48))
        vis = (qseg == kseg) & (qmem | kmem | (kidx <= qidx))
        return jnp.where(vis, 3e38, FILL).astype(F32)
    r = lax.broadcasted_iota(jnp.int32, (32, 48), 0)
    c = lax.broadcasted_iota(jnp.int32, (32, 48), 1)
    ce = cap(jnp.zeros_like(r), r < 8, r - 8, c)
    r = lax.broadcasted_iota(jnp.int32, (48, 80), 0)
    c = lax.broadcasted_iota(jnp.int32, (48, 80), 1)
    qseg = 1 - ((r >= 32) & (r < 40)).astype(jnp.int32)
    qidx = jnp.where(r < 16, r + 16, jnp.where(r < 40, r - 8, r - 40))
    co = cap(qseg, r < 8, qidx, c)
    return ce, co


def _softmax_p(s, cap):
    s = jnp.minimum(s, cap)
    m = jnp.max(s, axis=-1, keepdims=True)
    e = jnp.exp2((s - m) * EXP2_SCALE)
    l = jnp.sum(e, axis=-1, keepdims=True)
    return (e * pltpu.reciprocal(l, approx=True)).astype(BF)


def _bf(ref_u32, idx=...):
    return pltpu.bitcast(ref_u32[idx], BF)


def _transpose8(X):
    sub = lax.broadcasted_iota(jnp.int32, (8, 128), 0)
    X = list(X)
    for k in (4, 2, 1):
        m = (sub & k) != 0
        Y = list(X)
        for s in range(8):
            if not s & k:
                Y[s] = jnp.where(m, pltpu.roll(X[s + k], k, 0), X[s])
                Y[s + k] = jnp.where(m, X[s + k], pltpu.roll(X[s], 8 - k, 0))
        X = Y
    return X


def _ds(start, size, align):
    if not isinstance(start, int):
        start = pl.multiple_of(start, align)
    return pl.ds(start, size)


def _kernel(xT_hbm, mem0_hbm, wq_hbm, wk_hbm, wv_hbm, woT_hbm, w1_hbm, w2T_hbm,
            outT_hbm,
            xT_ref, mem0_ref, wst_ref, woT_ref, w1_ref, w2T_ref, outT_ref,
            xn_ref, xnu_ref, w_ref, wo_ref, w1u_ref, w2u_ref, orow_ref, act_ref,
            kg_ref, vg_ref, q8a_ref, q16_ref, q8b_ref, ce_ref, co_ref,
            sems, xsems, wsems, osem):
    def cp_x(b):
        cols = _ds(b * TB, TB, TB)
        return pltpu.make_async_copy(xT_hbm.at[:, cols], xT_ref.at[:, cols], xsems.at[b])

    cp_w1 = [pltpu.make_async_copy(w1_hbm.at[:, i * FH:(i + 1) * FH],
                                   w1_ref.at[:, i * FH:(i + 1) * FH], sems.at[i]) for i in range(2)]
    cp_m = pltpu.make_async_copy(mem0_hbm, mem0_ref, sems.at[2])
    cp_w2 = pltpu.make_async_copy(w2T_hbm, w2T_ref, sems.at[3])

    def cp_wo(i):
        heads = _ds(4 * i, 4, 4)
        return pltpu.make_async_copy(woT_hbm.at[heads], woT_ref.at[heads], sems.at[4 + i])

    def cp_w(g, mi):
        src = (wq_hbm, wk_hbm, wv_hbm)[mi // 2]
        c = mi % 2
        rows = _ds(g * GD * H, GD * H, GD * H)
        return pltpu.make_async_copy(src.at[rows, c * 128:(c + 1) * 128], wst_ref.at[mi, rows], wsems.at[g])

    def start_group(g):
        for mi in range(6):
            cp_w(g, mi).start()

    def wait_group(g):
        for mi in range(6):
            cp_w(g, mi).wait()

    def issue_a(k, c):
        pl.when(k == 0)(cp_x(0).start)
        pl.when(k == 1)(cp_w1[0].start)
        pl.when(k == 2)(cp_w1[1].start)

        @pl.when(k == 3)
        def _():
            cp_x(1).start()
            cp_x(2).start()
            cp_m.start()
        return c
    lax.fori_loop(0, 4, issue_a, 0)

    def issue_w(g, c):
        start_group(g)

        @pl.when(g + 3 < NB)
        def _():
            cp_x(g + 3).start()
        return c
    lax.fori_loop(0, NG, issue_w, 0)

    def issue_wo(i, c):
        pl.when(i == 2)(cp_w2.start)
        cp_wo(i).start()
        return c
    lax.fori_loop(0, 4, issue_wo, 0)

    ce, co = _caps()
    ce_ref[...] = ce
    co_ref[...] = co
    orow_ref[0:128, :] = jnp.zeros((128, D), F32)

    def ln(t0):
        x = xT_ref[:, _ds(t0, 128, 128)].astype(F32)
        mu = jnp.mean(x, axis=0, keepdims=True)
        xc = x - mu
        var = jnp.mean(xc * xc, axis=0, keepdims=True)
        xn = (xc / jnp.sqrt(var + 1e-5)).T
        xn_ref[_ds(t0, 128, 128), :] = xn
        xnu_ref[_ds(t0 // 2, 64, 64), :] = pltpu.bitcast(xn.astype(BF), U32)

    def silu_store(hf, t0, n, c0, c1):
        e = jnp.exp2(hf * (-LOG2E))
        act_ref[_ds(t0, n, n), c0:c1] = (hf * pltpu.reciprocal(1.0 + e, approx=True)).astype(BF)

    wst_u = wst_ref.bitcast(U32)

    def relayout_unit(g, cc, mi, c, m_lo, m_hi):
        d0 = g * GD + cc * 16
        blk = wst_u[2 * mi + c, _ds(d0 * 8, 128, 128), :]
        V = [blk[8 * d:8 * d + 8] for d in range(16)]
        lo = _transpose8([(V[2 * s] & m_lo) | (V[2 * s + 1] << 16) for s in range(8)])
        hi = _transpose8([(V[2 * s] >> 16) | (V[2 * s + 1] & m_hi) for s in range(8)])
        rows = _ds(g * (GD // 2) + cc * 8, 8, 8)
        for j in range(H // 2):
            col = 2 * j * 768 + mi * 256 + c * 128
            w_ref[rows, col:col + 128] = lo[j]
            w_ref[rows, col + 768:col + 896] = hi[j]

    def wo_unit(h):
        wo_ref[h * 128:(h + 1) * 128, :] = pltpu.bitcast(woT_ref[h].T, U32)

    def w2_unit(j):
        w2u_ref[j * 64:(j + 1) * 64, :] = pltpu.bitcast(w2T_ref[:, j * 128:(j + 1) * 128].T, U32)

    def pro_block(b, do_ln, g, z, extra=()):
        units = [(cc, mi, c) for cc in range(GD // 16) for mi in range(3) for c in range(2)]
        nsub, nslot = TB // MB, (TB // MB) * (F // 128)
        zero_v = jnp.full((8, 128), z, U32)
        k = 0
        for sb in range(nsub):
            ts = b * TB + sb * MB
            xb = _bf(xnu_ref, (_ds(ts // 2, MB // 2, MB // 2), slice(None)))
            hf = jnp.dot(xb, _bf(w1u_ref), preferred_element_type=F32)
            silu_store(hf, ts, MB, 0, F)
            while k < len(units) and (k * nslot) // len(units) < (sb + 1) * (F // 128):
                j = (k * nslot) // len(units) - sb * (F // 128)
                a = pltpu.bitcast(hf[0:8, j * 128:(j + 1) * 128], U32) & zero_v
                relayout_unit(g, *units[k], a | LO16, a | HI16)
                k += 1
            if sb == 0 and do_ln:
                for u in range(TB // 128):
                    ln((b + 1) * TB + u * 128)
            for h in extra[sb * len(extra) // nsub:(sb + 1) * len(extra) // nsub]:
                wo_unit(h)

    cp_x(0).wait()
    ln(0)
    ln(128)
    for i in range(2):
        cp_w1[i].wait()
        if i == 1:
            cp_x(1).wait()
        for u in range(TB // 128):
            xb = _bf(xnu_ref, (pl.ds(u * 64, 64), slice(None)))
            hf = jnp.dot(xb, w1_ref[:, i * FH:(i + 1) * FH], preferred_element_type=F32)
            silu_store(hf, u * 128, 128, i * FH, (i + 1) * FH)
            if i == 1:
                ln(TB + u * 128)
        w1u_ref[:, i * FH:(i + 1) * FH] = pltpu.bitcast(w1_ref[:, i * FH:(i + 1) * FH], U32)

    def pro_body(b, c):
        @pl.when(b + 1 < NB)
        def _():
            cp_x(b + 1).wait()
            wait_group(b - 1)
        z = lax.shift_right_logical(b, 10)
        pro_block(b, True, b - 1, z.astype(U32))
        return z
    z_last = lax.fori_loop(1, NB - 1, pro_body, jnp.int32(0))

    @pl.when(z_last == 0)
    def _():
        wait_group(NG - 1)
        cp_wo(0).wait()
    pro_block(NB - 1, False, NG - 1, z_last.astype(U32), extra=list(range(4)))

    def store_next(Rh, h, r0):
        hs = slice(h * 256, (h + 1) * 256)
        q8a_ref[:, hs] = Rh[r0:r0 + 8, 0:256]
        q16_ref[:, hs] = Rh[r0 + 8:r0 + 24, 0:256].astype(BF)
        q8b_ref[:, hs] = Rh[r0 + 24:r0 + 32, 0:256]
        kg_ref[:, hs] = Rh[r0:r0 + 32, 256:512].astype(BF)
        vg_ref[:, hs] = Rh[r0:r0 + 32, 512:768].astype(BF)

    def wcols(h, z):
        return _bf(w_ref, (pl.ds(z, D // 2), slice(h * 768, (h + 1) * 768)))

    lhs0 = xn_ref[0:32, :].astype(BF)
    WO = lambda a, b: [lambda h=h: wo_unit(h) for h in range(a, b)]
    W2 = lambda a, b: [lambda j=j: w2_unit(j) for j in range(a, b)]
    plan = [([cp_wo(1), cp_w2], range(0, 7), WO(4, 8) + W2(0, 9)),
            ([cp_wo(2)], range(7, 12), W2(9, 14) + WO(8, 12)),
            ([cp_wo(3), cp_m], range(12, 16), WO(12, 16))]
    for waits, heads, side in plan:
        @pl.when(z_last == 0)
        def _():
            for c in waits:
                c.wait()
        done = 0
        for n, h in enumerate(heads):
            store_next(jnp.dot(lhs0, wcols(h, 0), preferred_element_type=F32), h, 0)
            upto = (n + 1) * len(side) // len(heads)
            for fn in side[done:upto]:
                fn()
            done = upto

    def out_block(t0):
        cols = _ds(t0, 128, 128)
        y = orow_ref[cols, :].T
        outT_ref[:, cols] = (xT_ref[:, cols].astype(F32) + y).astype(BF)

    def cp_out(t0):
        cols = _ds(t0, 128, 128)
        return pltpu.make_async_copy(outT_ref.at[:, cols], outT_hbm.at[:, cols], osem)

    def pair(p, mem, sub, last=False):
        if isinstance(p, int):
            base, nxt, zsrc, zsh = p * 64, p * 64 + 64, z_last, 1
        else:
            base = pl.multiple_of(p * 64, 64)
            nxt, zsrc, zsh = pl.multiple_of(base + 64, 64), p, 10
        z = [pl.multiple_of(lax.shift_right_logical(zsrc, zsh + i + 2 * sub) * 8, 8) for i in range(2)]
        cap = (ce_ref[...], co_ref[...])
        FF = []

        def ffn2(j0, j1):
            a = act_ref[pl.ds(base, 64), j0 * 128:j1 * 128]
            FF.append(jnp.dot(a, _bf(w2u_ref, (slice(j0 * 64, j1 * 64), slice(None))),
                              preferred_element_type=F32))

        def out_proj(o, e):
            return jnp.dot(jnp.concatenate(o, axis=1), _bf(wo_ref, (pl.ds(z[e], H * DH // 2), slice(None))),
                           preferred_element_type=F32)

        lhs = jnp.concatenate([mem, xn_ref[pl.ds(base + 32, 24), :]], axis=0).astype(BF)
        R = [jnp.dot(lhs, wcols(h, z[0]), preferred_element_type=F32) for h in range(H)]
        keep, sc = [], []
        for h in range(H):
            hs = slice(h * 256, (h + 1) * 256)
            gb = R[h][16:32, :].astype(BF)
            gkv = R[h][0:16, 256:768].astype(BF)
            q = jnp.concatenate([
                jnp.concatenate([R[h][0:8, 0:256], q8a_ref[:, hs]], axis=0).astype(BF),
                q16_ref[:, hs]], axis=0)
            k = jnp.concatenate([kg_ref[:, hs], gkv[:, 0:256]], axis=0)
            keep.append((R[h][8:16, 0:256], gkv, gb))
            sc.append(lax.dot_general(q, k, NT, preferred_element_type=F32))
        ffn2(0, 4)
        o = []
        for h in range(H):
            v = jnp.concatenate([vg_ref[:, h * 256:(h + 1) * 256], keep[h][1][:, 256:512]], axis=0)
            o.append(jnp.dot(_softmax_p(sc[h], cap[0]), v, preferred_element_type=F32).astype(BF))
        Ce = out_proj(o, 0)
        ffn2(4, 7)

        parts = [Ce[0:8], xn_ref[pl.ds(base + 56, 8), :]]
        if not last:
            parts.append(xn_ref[pl.ds(nxt, 32), :])
        lhs = jnp.concatenate(parts, axis=0).astype(BF)
        R = [jnp.dot(lhs, wcols(h, z[1]), preferred_element_type=F32) for h in range(H)]
        gcs, sc = [], []
        for h in range(H):
            hs = slice(h * 256, (h + 1) * 256)
            qa, gkv, gb = keep[h]
            gc = R[h][0:16, :].astype(BF)
            q = jnp.concatenate([
                gc[:, 0:256], gb[:, 0:256],
                jnp.concatenate([q8b_ref[:, hs], qa], axis=0).astype(BF)], axis=0)
            k = jnp.concatenate([kg_ref[:, hs], gkv[:, 0:256], gb[:, 256:512], gc[:, 256:512]], axis=0)
            gcs.append(gc)
            sc.append(lax.dot_general(q, k, NT, preferred_element_type=F32))
        ffn2(7, 11)
        o = []
        for h in range(H):
            _, gkv, gb = keep[h]
            v = jnp.concatenate([vg_ref[:, h * 256:(h + 1) * 256], gkv[:, 256:512], gb[:, 512:768],
                                 gcs[h][:, 512:768]], axis=0)
            o.append(jnp.dot(_softmax_p(sc[h], cap[1]), v, preferred_element_type=F32).astype(BF))
        Co = out_proj(o, 1)
        if not last:
            for h in range(H):
                store_next(R[h], h, 16)
        ffn2(11, 14)

        tot = jnp.concatenate([Ce[8:32], Co[32:40], Co[40:48], Co[16:32], Co[8:16]], axis=0)
        for f in FF:
            tot = tot + f
        orow_ref[pl.ds(base, 64), :] = tot
        return Co[0:8]

    def body(i, mem):
        if isinstance(i, int):
            tprev = (i - 1) * 128
            out_block(tprev)
            cp_out(tprev).start()
        else:
            tprev = jnp.maximum(i - 1, 0) * 128
            out_block(tprev)

            @pl.when(i > 0)
            def _():
                cp_out(tprev).start()
        mem = pair(2 * i, mem, 0)
        return pair(2 * i + 1, mem, 1, last=isinstance(i, int))
    mem = lax.fori_loop(0, NPAIR // 2 - 1, body, mem0_ref[...].astype(F32))
    body(NPAIR // 2 - 1, mem)

    out_block(S - 128)
    cp_out(S - 128).start()
    for b in range(S // 128):
        cp_out(b * 128).wait()


@jax.jit
def pallas_parallel_sum__memory_aug_recurrent_mem_tr__dense_activation_silu__prompt_kernel(
    A_x, A_mem0, A_Wq, A_Wk, A_Wv, A_Wo, A_seg_len, B_x, B_w1, B_w2,
):
    hbm = pl.BlockSpec(memory_space=pltpu.HBM)
    outT = pl.pallas_call(
        _kernel,
        out_shape=jax.ShapeDtypeStruct((D, S), BF),
        in_specs=[hbm] * 8,
        out_specs=hbm,
        scratch_shapes=[
            pltpu.VMEM((D, S), BF),
            pltpu.VMEM((M, D), BF),
            pltpu.VMEM((6, D * H, 128), BF),
            pltpu.VMEM((H, D, DH), BF),
            pltpu.VMEM((D, F), BF),
            pltpu.VMEM((D, F), BF),
            pltpu.VMEM((D, S), BF),
            pltpu.VMEM((S, D), F32),
            pltpu.VMEM((S // 2, D), U32),
            pltpu.VMEM((D // 2, 3 * H * DH), U32),
            pltpu.VMEM((H * DH // 2, D), U32),
            pltpu.VMEM((D // 2, F), U32),
            pltpu.VMEM((F // 2, D), U32),
            pltpu.VMEM((S, D), F32),
            pltpu.VMEM((S, F), BF),
            pltpu.VMEM((32, H * DH), BF),
            pltpu.VMEM((32, H * DH), BF),
            pltpu.VMEM((8, H * DH), F32),
            pltpu.VMEM((16, H * DH), BF),
            pltpu.VMEM((8, H * DH), F32),
            pltpu.VMEM((32, 48), F32),
            pltpu.VMEM((48, 80), F32),
            pltpu.SemaphoreType.DMA((8,)),
            pltpu.SemaphoreType.DMA((NB,)),
            pltpu.SemaphoreType.DMA((NG,)),
            pltpu.SemaphoreType.DMA(()),
        ],
        compiler_params=pltpu.CompilerParams(vmem_limit_bytes=110 * 1024 * 1024),
    )(jnp.swapaxes(A_x, 1, 2).reshape(D, S), A_mem0.reshape(M, D),
      A_Wq.reshape(D * H, DH), A_Wk.reshape(D * H, DH), A_Wv.reshape(D * H, DH),
      jnp.swapaxes(A_Wo, 1, 2), B_w1, B_w2.T)
    return jnp.swapaxes(outT.reshape(1, D, S), 1, 2)
```

```python
import jax
import jax.numpy as jnp
import numpy as np
from jax import lax
import jax.experimental.pallas as pl
import jax.experimental.pallas.tpu as pltpu

S, D, H, DH, M, SEG, F = 2048, 448, 16, 256, 8, 32, 1792
NPAIR = S // (2 * SEG)
TB = 256
NB = S // TB
MB = 64
GD = 64
NG = D // GD
FH = F // 2
BF, F32, U32 = jnp.bfloat16, jnp.float32, jnp.uint32
LOG2E = float(np.log2(np.e))
EXP2_SCALE = float(DH ** -0.5 * LOG2E)
FILL = -1e9 * DH ** 0.5
NT = (((1,), (1,)), ((), ()))
LO16, HI16 = np.uint32(0x0000FFFF), np.uint32(0xFFFF0000)


def _caps():
    def cap(qseg, qmem, qidx, c):
        kseg = (c >= 40).astype(jnp.int32)
        kmem = ((c >= 32) & (c < 40)) | ((c >= 64) & (c < 72))
        kidx = jnp.where(c < 32, c, jnp.where(c < 64, c - 40, c - 48))
        vis = (qseg == kseg) & (qmem | kmem | (kidx <= qidx))
        return jnp.where(vis, 3e38, FILL).astype(F32)
    r = lax.broadcasted_iota(jnp.int32, (32, 48), 0)
    c = lax.broadcasted_iota(jnp.int32, (32, 48), 1)
    ce = cap(jnp.zeros_like(r), r < 8, r - 8, c)
    r = lax.broadcasted_iota(jnp.int32, (48, 80), 0)
    c = lax.broadcasted_iota(jnp.int32, (48, 80), 1)
    qseg = 1 - ((r >= 32) & (r < 40)).astype(jnp.int32)
    qidx = jnp.where(r < 16, r + 16, jnp.where(r < 40, r - 8, r - 40))
    co = cap(qseg, r < 8, qidx, c)
    return ce, co


def _softmax_p(s, cap):
    s = jnp.minimum(s, cap)
    m = jnp.max(s, axis=-1, keepdims=True)
    e = jnp.exp2((s - m) * EXP2_SCALE)
    l = jnp.sum(e, axis=-1, keepdims=True)
    return (e * pltpu.reciprocal(l, approx=True)).astype(BF)


def _bf(ref_u32, idx=...):
    return pltpu.bitcast(ref_u32[idx], BF)


def _transpose8(X):
    sub = lax.broadcasted_iota(jnp.int32, (8, 128), 0)
    X = list(X)
    for k in (4, 2, 1):
        m = (sub & k) != 0
        Y = list(X)
        for s in range(8):
            if not s & k:
                Y[s] = jnp.where(m, pltpu.roll(X[s + k], k, 0), X[s])
                Y[s + k] = jnp.where(m, X[s + k], pltpu.roll(X[s], 8 - k, 0))
        X = Y
    return X


def _ds(start, size, align):
    if not isinstance(start, int):
        start = pl.multiple_of(start, align)
    return pl.ds(start, size)


def _kernel(xT_hbm, mem0_hbm, wq_hbm, wk_hbm, wv_hbm, woT_hbm, w1_hbm, w2T_hbm,
            outT_hbm,
            xT_ref, mem0_ref, wst_ref, woT_ref, w1_ref, w2T_ref, outT_ref,
            xn_ref, xnu_ref, w_ref, wo_ref, w1u_ref, w2u_ref, orow_ref, act_ref,
            kg_ref, vg_ref, q8a_ref, q16_ref, q8b_ref, ce_ref, co_ref,
            sems, xsems, wsems, osem):
    def cp_x(b):
        cols = _ds(b * TB, TB, TB)
        return pltpu.make_async_copy(xT_hbm.at[:, cols], xT_ref.at[:, cols], xsems.at[b])

    cp_w1 = [pltpu.make_async_copy(w1_hbm.at[:, i * FH:(i + 1) * FH],
                                   w1_ref.at[:, i * FH:(i + 1) * FH], sems.at[i]) for i in range(2)]
    cp_m = pltpu.make_async_copy(mem0_hbm, mem0_ref, sems.at[2])
    cp_w2 = pltpu.make_async_copy(w2T_hbm, w2T_ref, sems.at[3])

    def cp_wo(i):
        heads = _ds(4 * i, 4, 4)
        return pltpu.make_async_copy(woT_hbm.at[heads], woT_ref.at[heads], sems.at[4 + i])

    def cp_w(g, mi):
        src = (wq_hbm, wk_hbm, wv_hbm)[mi // 2]
        c = mi % 2
        rows = _ds(g * GD * H, GD * H, GD * H)
        return pltpu.make_async_copy(src.at[rows, c * 128:(c + 1) * 128], wst_ref.at[mi, rows], wsems.at[g])

    def start_group(g):
        for mi in range(6):
            cp_w(g, mi).start()

    def wait_group(g):
        for mi in range(6):
            cp_w(g, mi).wait()

    def issue_a(k, c):
        pl.when(k == 0)(cp_x(0).start)
        pl.when(k == 1)(cp_w1[0].start)
        pl.when(k == 2)(cp_w1[1].start)

        @pl.when(k == 3)
        def _():
            cp_x(1).start()
            cp_x(2).start()
            cp_m.start()
        return c
    lax.fori_loop(0, 4, issue_a, 0)

    def issue_w(g, c):
        start_group(g)

        @pl.when(g + 3 < NB)
        def _():
            cp_x(g + 3).start()
        return c
    lax.fori_loop(0, NG, issue_w, 0)

    def issue_wo(i, c):
        pl.when(i == 2)(cp_w2.start)
        cp_wo(i).start()
        return c
    lax.fori_loop(0, 4, issue_wo, 0)

    ce, co = _caps()
    ce_ref[...] = ce
    co_ref[...] = co
    orow_ref[0:128, :] = jnp.zeros((128, D), F32)

    def ln(t0):
        x = xT_ref[:, _ds(t0, 128, 128)].astype(F32)
        mu = jnp.mean(x, axis=0, keepdims=True)
        xc = x - mu
        var = jnp.mean(xc * xc, axis=0, keepdims=True)
        xn = (xc / jnp.sqrt(var + 1e-5)).T
        xn_ref[_ds(t0, 128, 128), :] = xn
        xnu_ref[_ds(t0 // 2, 64, 64), :] = pltpu.bitcast(xn.astype(BF), U32)

    def silu_store(hf, t0, n, c0, c1):
        e = jnp.exp2(hf * (-LOG2E))
        act_ref[_ds(t0, n, n), c0:c1] = (hf * pltpu.reciprocal(1.0 + e, approx=True)).astype(BF)

    wst_u = wst_ref.bitcast(U32)

    def relayout_unit(g, cc, mi, c, m_lo, m_hi):
        d0 = g * GD + cc * 16
        blk = wst_u[2 * mi + c, _ds(d0 * 8, 128, 128), :]
        V = [blk[8 * d:8 * d + 8] for d in range(16)]
        lo = _transpose8([(V[2 * s] & m_lo) | (V[2 * s + 1] << 16) for s in range(8)])
        hi = _transpose8([(V[2 * s] >> 16) | (V[2 * s + 1] & m_hi) for s in range(8)])
        rows = _ds(g * (GD // 2) + cc * 8, 8, 8)
        for j in range(H // 2):
            col = 2 * j * 768 + mi * 256 + c * 128
            w_ref[rows, col:col + 128] = lo[j]
            w_ref[rows, col + 768:col + 896] = hi[j]

    def wo_unit(h):
        wo_ref[h * 128:(h + 1) * 128, :] = pltpu.bitcast(woT_ref[h].T, U32)

    def w2_unit(j):
        w2u_ref[j * 64:(j + 1) * 64, :] = pltpu.bitcast(w2T_ref[:, j * 128:(j + 1) * 128].T, U32)

    def pro_block(b, do_ln, g, z, extra=()):
        units = [(cc, mi, c) for cc in range(GD // 16) for mi in range(3) for c in range(2)]
        nsub, nslot = TB // MB, (TB // MB) * (F // 128)
        zero_v = jnp.full((8, 128), z, U32)
        k = 0
        for sb in range(nsub):
            ts = b * TB + sb * MB
            xb = _bf(xnu_ref, (_ds(ts // 2, MB // 2, MB // 2), slice(None)))
            hf = jnp.dot(xb, _bf(w1u_ref), preferred_element_type=F32)
            silu_store(hf, ts, MB, 0, F)
            while k < len(units) and (k * nslot) // len(units) < (sb + 1) * (F // 128):
                j = (k * nslot) // len(units) - sb * (F // 128)
                a = pltpu.bitcast(hf[0:8, j * 128:(j + 1) * 128], U32) & zero_v
                relayout_unit(g, *units[k], a | LO16, a | HI16)
                k += 1
            if sb == 0 and do_ln:
                for u in range(TB // 128):
                    ln((b + 1) * TB + u * 128)
            for h in extra[sb * len(extra) // nsub:(sb + 1) * len(extra) // nsub]:
                wo_unit(h)

    cp_x(0).wait()
    ln(0)
    ln(128)
    for i in range(2):
        cp_w1[i].wait()
        if i == 1:
            cp_x(1).wait()
        for u in range(TB // 128):
            xb = _bf(xnu_ref, (pl.ds(u * 64, 64), slice(None)))
            hf = jnp.dot(xb, w1_ref[:, i * FH:(i + 1) * FH], preferred_element_type=F32)
            silu_store(hf, u * 128, 128, i * FH, (i + 1) * FH)
            if i == 1:
                ln(TB + u * 128)
        w1u_ref[:, i * FH:(i + 1) * FH] = pltpu.bitcast(w1_ref[:, i * FH:(i + 1) * FH], U32)

    def pro_body(b, c):
        @pl.when(b + 1 < NB)
        def _():
            cp_x(b + 1).wait()
            wait_group(b - 1)
        z = lax.shift_right_logical(b, 10)
        pro_block(b, True, b - 1, z.astype(U32))
        return z
    z_last = lax.fori_loop(1, NB - 1, pro_body, jnp.int32(0))

    @pl.when(z_last == 0)
    def _():
        wait_group(NG - 1)
        cp_wo(0).wait()
    pro_block(NB - 1, False, NG - 1, z_last.astype(U32), extra=list(range(4)))

    def store_next(Rh, h, r0):
        hs = slice(h * 256, (h + 1) * 256)
        q8a_ref[:, hs] = Rh[r0:r0 + 8, 0:256]
        q16_ref[:, hs] = Rh[r0 + 8:r0 + 24, 0:256].astype(BF)
        q8b_ref[:, hs] = Rh[r0 + 24:r0 + 32, 0:256]
        kg_ref[:, hs] = Rh[r0:r0 + 32, 256:512].astype(BF)
        vg_ref[:, hs] = Rh[r0:r0 + 32, 512:768].astype(BF)

    def wcols(h, z):
        return _bf(w_ref, (pl.ds(z, D // 2), slice(h * 768, (h + 1) * 768)))

    lhs0 = xn_ref[0:32, :].astype(BF)
    WO = lambda a, b: [lambda h=h: wo_unit(h) for h in range(a, b)]
    W2 = lambda a, b: [lambda j=j: w2_unit(j) for j in range(a, b)]
    plan = [([cp_wo(1), cp_w2], range(0, 7), WO(4, 8) + W2(0, 9)),
            ([cp_wo(2)], range(7, 12), W2(9, 14) + WO(8, 12)),
            ([cp_wo(3), cp_m], range(12, 16), WO(12, 16))]
    for waits, heads, side in plan:
        @pl.when(z_last == 0)
        def _():
            for c in waits:
                c.wait()
        done = 0
        for n, h in enumerate(heads):
            store_next(jnp.dot(lhs0, wcols(h, 0), preferred_element_type=F32), h, 0)
            upto = (n + 1) * len(side) // len(heads)
            for fn in side[done:upto]:
                fn()
            done = upto

    def out_block(t0, z=None):
        cols = _ds(t0, 128, 128)
        y = xT_ref[:, cols].astype(F32) + orow_ref[cols, :].T
        outT_ref[:, cols] = y.astype(BF)
        if z is None:
            return None
        bits = pltpu.bitcast(y, U32)
        acc = bits[0:8]
        for r in range(8, D, 8):
            acc = acc | bits[r:r + 8]
        return acc & jnp.full((8, 128), z, U32)

    def pin(mem, dep):
        head = pltpu.bitcast(pltpu.bitcast(mem[:, 0:128], U32) | dep, F32)
        return jnp.concatenate([head, mem[:, 128:]], axis=1)

    def cp_out(t0):
        cols = _ds(t0, 128, 128)
        return pltpu.make_async_copy(outT_ref.at[:, cols], outT_hbm.at[:, cols], osem)

    def pair(p, mem, sub, last=False):
        if isinstance(p, int):
            base, nxt, zsrc, zsh = p * 64, p * 64 + 64, z_last, 1
        else:
            base = pl.multiple_of(p * 64, 64)
            nxt, zsrc, zsh = pl.multiple_of(base + 64, 64), p, 10
        z = [pl.multiple_of(lax.shift_right_logical(zsrc, zsh + i + 2 * sub) * 8, 8) for i in range(2)]
        cap = (ce_ref[...], co_ref[...])
        FF = []

        def ffn2(j0, j1):
            a = act_ref[pl.ds(base, 64), j0 * 128:j1 * 128]
            FF.append(jnp.dot(a, _bf(w2u_ref, (slice(j0 * 64, j1 * 64), slice(None))),
                              preferred_element_type=F32))

        def out_proj(o, e):
            return jnp.dot(jnp.concatenate(o, axis=1), _bf(wo_ref, (pl.ds(z[e], H * DH // 2), slice(None))),
                           preferred_element_type=F32)

        lhs = jnp.concatenate([mem, xn_ref[pl.ds(base + 32, 24), :]], axis=0).astype(BF)
        R = [jnp.dot(lhs, wcols(h, z[0]), preferred_element_type=F32) for h in range(H)]
        keep, sc = [], []
        for h in range(H):
            hs = slice(h * 256, (h + 1) * 256)
            gb = R[h][16:32, :].astype(BF)
            gkv = R[h][0:16, 256:768].astype(BF)
            q = jnp.concatenate([
                jnp.concatenate([R[h][0:8, 0:256], q8a_ref[:, hs]], axis=0).astype(BF),
                q16_ref[:, hs]], axis=0)
            k = jnp.concatenate([kg_ref[:, hs], gkv[:, 0:256]], axis=0)
            keep.append((R[h][8:16, 0:256], gkv, gb))
            sc.append(lax.dot_general(q, k, NT, preferred_element_type=F32))
        ffn2(0, 4)
        o = []
        for h in range(H):
            v = jnp.concatenate([vg_ref[:, h * 256:(h + 1) * 256], keep[h][1][:, 256:512]], axis=0)
            o.append(jnp.dot(_softmax_p(sc[h], cap[0]), v, preferred_element_type=F32).astype(BF))
        Ce = out_proj(o, 0)
        ffn2(4, 7)

        parts = [Ce[0:8], xn_ref[pl.ds(base + 56, 8), :]]
        if not last:
            parts.append(xn_ref[pl.ds(nxt, 32), :])
        lhs = jnp.concatenate(parts, axis=0).astype(BF)
        R = [jnp.dot(lhs, wcols(h, z[1]), preferred_element_type=F32) for h in range(H)]
        gcs, sc = [], []
        for h in range(H):
            hs = slice(h * 256, (h + 1) * 256)
            qa, gkv, gb = keep[h]
            gc = R[h][0:16, :].astype(BF)
            q = jnp.concatenate([
                gc[:, 0:256], gb[:, 0:256],
                jnp.concatenate([q8b_ref[:, hs], qa], axis=0).astype(BF)], axis=0)
            k = jnp.concatenate([kg_ref[:, hs], gkv[:, 0:256], gb[:, 256:512], gc[:, 256:512]], axis=0)
            gcs.append(gc)
            sc.append(lax.dot_general(q, k, NT, preferred_element_type=F32))
        ffn2(7, 11)
        o = []
        for h in range(H):
            _, gkv, gb = keep[h]
            v = jnp.concatenate([vg_ref[:, h * 256:(h + 1) * 256], gkv[:, 256:512], gb[:, 512:768],
                                 gcs[h][:, 512:768]], axis=0)
            o.append(jnp.dot(_softmax_p(sc[h], cap[1]), v, preferred_element_type=F32).astype(BF))
        Co = out_proj(o, 1)
        if not last:
            for h in range(H):
                store_next(R[h], h, 16)
        ffn2(11, 13)
        ffn2(13, 14)

        tot = jnp.concatenate([Ce[8:32], Co[32:40], Co[40:48], Co[16:32], Co[8:16]], axis=0)
        for f in FF:
            tot = tot + f
        orow_ref[pl.ds(base, 64), :] = tot
        return Co[0:8]

    def body(i, mem):
        if isinstance(i, int):
            tprev = (i - 1) * 128
            out_block(tprev)
            cp_out(tprev).start()
        else:
            tprev = jnp.maximum(i - 1, 0) * 128
            dep = out_block(tprev, lax.shift_right_logical(i, 10).astype(U32))

            @pl.when(i > 0)
            def _():
                cp_out(tprev).start()
        mem = pair(2 * i, mem, 0)
        if not isinstance(i, int):
            mem = pin(mem, dep)
        return pair(2 * i + 1, mem, 1, last=isinstance(i, int))
    mem = lax.fori_loop(0, NPAIR // 2 - 1, body, mem0_ref[...].astype(F32))
    body(NPAIR // 2 - 1, mem)

    out_block(S - 128)
    cp_out(S - 128).start()
    for b in range(S // 128):
        cp_out(b * 128).wait()


@jax.jit
def pallas_parallel_sum__memory_aug_recurrent_mem_tr__dense_activation_silu__prompt_kernel(
    A_x, A_mem0, A_Wq, A_Wk, A_Wv, A_Wo, A_seg_len, B_x, B_w1, B_w2,
):
    hbm = pl.BlockSpec(memory_space=pltpu.HBM)
    outT = pl.pallas_call(
        _kernel,
        out_shape=jax.ShapeDtypeStruct((D, S), BF),
        in_specs=[hbm] * 8,
        out_specs=hbm,
        scratch_shapes=[
            pltpu.VMEM((D, S), BF),
            pltpu.VMEM((M, D), BF),
            pltpu.VMEM((6, D * H, 128), BF),
            pltpu.VMEM((H, D, DH), BF),
            pltpu.VMEM((D, F), BF),
            pltpu.VMEM((D, F), BF),
            pltpu.VMEM((D, S), BF),
            pltpu.VMEM((S, D), F32),
            pltpu.VMEM((S // 2, D), U32),
            pltpu.VMEM((D // 2, 3 * H * DH), U32),
            pltpu.VMEM((H * DH // 2, D), U32),
            pltpu.VMEM((D // 2, F), U32),
            pltpu.VMEM((F // 2, D), U32),
            pltpu.VMEM((S, D), F32),
            pltpu.VMEM((S, F), BF),
            pltpu.VMEM((32, H * DH), BF),
            pltpu.VMEM((32, H * DH), BF),
            pltpu.VMEM((8, H * DH), F32),
            pltpu.VMEM((16, H * DH), BF),
            pltpu.VMEM((8, H * DH), F32),
            pltpu.VMEM((32, 48), F32),
            pltpu.VMEM((48, 80), F32),
            pltpu.SemaphoreType.DMA((8,)),
            pltpu.SemaphoreType.DMA((NB,)),
            pltpu.SemaphoreType.DMA((NG,)),
            pltpu.SemaphoreType.DMA(()),
        ],
        compiler_params=pltpu.CompilerParams(vmem_limit_bytes=110 * 1024 * 1024),
    )(jnp.swapaxes(A_x, 1, 2).reshape(D, S), A_mem0.reshape(M, D),
      A_Wq.reshape(D * H, DH), A_Wk.reshape(D * H, DH), A_Wv.reshape(D * H, DH),
      jnp.swapaxes(A_Wo, 1, 2), B_w1, B_w2.T)
    return jnp.swapaxes(outT.reshape(1, D, S), 1, 2)
```

```python
import jax
import jax.numpy as jnp
import numpy as np
from jax import lax
import jax.experimental.pallas as pl
import jax.experimental.pallas.tpu as pltpu

S, D, H, DH, M, SEG, F = 2048, 448, 16, 256, 8, 32, 1792
NPAIR = S // (2 * SEG)
TB = 256
NB = S // TB
MB = 64
GD = 64
NG = D // GD
FH = F // 2
BF, F32, U32 = jnp.bfloat16, jnp.float32, jnp.uint32
LOG2E = float(np.log2(np.e))
EXP2_SCALE = float(DH ** -0.5 * LOG2E)
FILL = -1e9 * DH ** 0.5
NT = (((1,), (1,)), ((), ()))
LO16, HI16 = np.uint32(0x0000FFFF), np.uint32(0xFFFF0000)


def _caps():
    def cap(qseg, qmem, qidx, c):
        kseg = (c >= 40).astype(jnp.int32)
        kmem = ((c >= 32) & (c < 40)) | ((c >= 64) & (c < 72))
        kidx = jnp.where(c < 32, c, jnp.where(c < 64, c - 40, c - 48))
        vis = (qseg == kseg) & (qmem | kmem | (kidx <= qidx))
        return jnp.where(vis, 3e38, FILL).astype(F32)
    r = lax.broadcasted_iota(jnp.int32, (32, 48), 0)
    c = lax.broadcasted_iota(jnp.int32, (32, 48), 1)
    ce = cap(jnp.zeros_like(r), r < 8, r - 8, c)
    r = lax.broadcasted_iota(jnp.int32, (48, 80), 0)
    c = lax.broadcasted_iota(jnp.int32, (48, 80), 1)
    qseg = 1 - ((r >= 32) & (r < 40)).astype(jnp.int32)
    qidx = jnp.where(r < 16, r + 16, jnp.where(r < 40, r - 8, r - 40))
    co = cap(qseg, r < 8, qidx, c)
    return ce, co


def _softmax_p(s, cap):
    s = jnp.minimum(s, cap)
    m = jnp.max(s, axis=-1, keepdims=True)
    e = jnp.exp2((s - m) * EXP2_SCALE)
    l = jnp.sum(e, axis=-1, keepdims=True)
    return (e * pltpu.reciprocal(l, approx=True)).astype(BF)


def _bf(ref_u32, idx=...):
    return pltpu.bitcast(ref_u32[idx], BF)


def _transpose8(X):
    sub = lax.broadcasted_iota(jnp.int32, (8, 128), 0)
    X = list(X)
    for k in (4, 2, 1):
        m = (sub & k) != 0
        Y = list(X)
        for s in range(8):
            if not s & k:
                Y[s] = jnp.where(m, pltpu.roll(X[s + k], k, 0), X[s])
                Y[s + k] = jnp.where(m, X[s + k], pltpu.roll(X[s], 8 - k, 0))
        X = Y
    return X


def _ds(start, size, align):
    if not isinstance(start, int):
        start = pl.multiple_of(start, align)
    return pl.ds(start, size)


def _kernel(xT_hbm, mem0_hbm, wq_hbm, wk_hbm, wv_hbm, woT_hbm, w1_hbm, w2T_hbm,
            outT_hbm,
            xT_ref, mem0_ref, wst_ref, woT_ref, w1_ref, w2T_ref, outT_ref,
            xn_ref, xnu_ref, w_ref, wo_ref, w1u_ref, w2u_ref, orow_ref, act_ref,
            kg_ref, vg_ref, q8a_ref, q16_ref, q8b_ref, ce_ref, co_ref,
            sems, xsems, wsems, osem):
    def cp_x(b):
        cols = _ds(b * TB, TB, TB)
        return pltpu.make_async_copy(xT_hbm.at[:, cols], xT_ref.at[:, cols], xsems.at[b])

    cp_w1 = [pltpu.make_async_copy(w1_hbm.at[:, i * FH:(i + 1) * FH],
                                   w1_ref.at[:, i * FH:(i + 1) * FH], sems.at[i]) for i in range(2)]
    cp_m = pltpu.make_async_copy(mem0_hbm, mem0_ref, sems.at[2])
    cp_w2 = pltpu.make_async_copy(w2T_hbm, w2T_ref, sems.at[3])

    def cp_wo(i):
        heads = slice(4 * i, 4 * i + 4)
        return pltpu.make_async_copy(woT_hbm.at[heads], woT_ref.at[heads], sems.at[4 + i])

    def cp_w(g, mi):
        src = (wq_hbm, wk_hbm, wv_hbm)[mi // 2]
        c = mi % 2
        rows = _ds(g * GD * H, GD * H, GD * H)
        return pltpu.make_async_copy(src.at[rows, c * 128:(c + 1) * 128], wst_ref.at[mi, rows], wsems.at[g])

    def start_group(g):
        for mi in range(6):
            cp_w(g, mi).start()

    def wait_group(g):
        for mi in range(6):
            cp_w(g, mi).wait()

    def issue_a(k, c):
        pl.when(k == 0)(cp_x(0).start)
        pl.when(k == 1)(cp_w1[0].start)
        pl.when(k == 2)(cp_w1[1].start)

        @pl.when(k == 3)
        def _():
            cp_x(1).start()
            cp_x(2).start()
            cp_m.start()
        return c
    lax.fori_loop(0, 4, issue_a, 0)

    def issue_w(g, c):
        start_group(g)

        @pl.when(g + 3 < NB)
        def _():
            cp_x(g + 3).start()
        return c
    lax.fori_loop(0, NG, issue_w, 0)

    def issue_wo(k, c):
        pl.when(k == 0)(cp_w2.start)
        for i in range(4):
            pl.when(k == i + 1)(cp_wo(i).start)
        return c
    lax.fori_loop(0, 5, issue_wo, 0)

    ce, co = _caps()
    ce_ref[...] = ce
    co_ref[...] = co
    orow_ref[0:128, :] = jnp.zeros((128, D), F32)

    def ln(t0):
        x = xT_ref[:, _ds(t0, 128, 128)].astype(F32)
        mu = jnp.mean(x, axis=0, keepdims=True)
        xc = x - mu
        var = jnp.mean(xc * xc, axis=0, keepdims=True)
        xn = (xc / jnp.sqrt(var + 1e-5)).T
        xn_ref[_ds(t0, 128, 128), :] = xn
        xnu_ref[_ds(t0 // 2, 64, 64), :] = pltpu.bitcast(xn.astype(BF), U32)

    def silu_store(hf, t0, n, c0, c1):
        e = jnp.exp2(hf * (-LOG2E))
        act_ref[_ds(t0, n, n), c0:c1] = (hf * pltpu.reciprocal(1.0 + e, approx=True)).astype(BF)

    def relayout_unit(g, cc, mi, c, m_lo, m_hi):
        d0 = g * GD + cc * 16
        blk = pltpu.bitcast(wst_ref[2 * mi + c, _ds(d0 * H, 256, 256), :], U32)
        V = [blk[8 * d:8 * d + 8] for d in range(16)]
        lo = _transpose8([(V[2 * s] & m_lo) | (V[2 * s + 1] << 16) for s in range(8)])
        hi = _transpose8([(V[2 * s] >> 16) | (V[2 * s + 1] & m_hi) for s in range(8)])
        rows = _ds(g * (GD // 2) + cc * 8, 8, 8)
        for j in range(H // 2):
            col = 2 * j * 768 + mi * 256 + c * 128
            w_ref[rows, col:col + 128] = lo[j]
            w_ref[rows, col + 768:col + 896] = hi[j]

    def wo_unit(h):
        wo_ref[h * 128:(h + 1) * 128, :] = pltpu.bitcast(woT_ref[h].T, U32)

    def w2_unit(j):
        w2u_ref[j * 64:(j + 1) * 64, :] = pltpu.bitcast(w2T_ref[:, j * 128:(j + 1) * 128].T, U32)

    def pro_block(b, do_ln, g, z, extra=()):
        units = [(cc, mi, c) for cc in range(GD // 16) for mi in range(3) for c in range(2)]
        nsub, nslot = TB // MB, (TB // MB) * (F // 128)
        zero_v = jnp.full((8, 128), z, U32)
        k = 0
        for sb in range(nsub):
            ts = b * TB + sb * MB
            xb = _bf(xnu_ref, (_ds(ts // 2, MB // 2, MB // 2), slice(None)))
            hf = jnp.dot(xb, _bf(w1u_ref), preferred_element_type=F32)
            silu_store(hf, ts, MB, 0, F)
            while k < len(units) and (k * nslot) // len(units) < (sb + 1) * (F // 128):
                j = (k * nslot) // len(units) - sb * (F // 128)
                a = pltpu.bitcast(hf[0:8, j * 128:(j + 1) * 128], U32) & zero_v
                relayout_unit(g, *units[k], a | LO16, a | HI16)
                k += 1
            if sb == 0 and do_ln:
                for u in range(TB // 128):
                    ln((b + 1) * TB + u * 128)
            for j in extra[sb * len(extra) // nsub:(sb + 1) * len(extra) // nsub]:
                w2_unit(j)

    cp_x(0).wait()
    ln(0)
    ln(128)
    for i in range(2):
        cp_w1[i].wait()
        if i == 1:
            cp_x(1).wait()
        for u in range(TB // 128):
            xb = _bf(xnu_ref, (pl.ds(u * 64, 64), slice(None)))
            hf = jnp.dot(xb, w1_ref[:, i * FH:(i + 1) * FH], preferred_element_type=F32)
            silu_store(hf, u * 128, 128, i * FH, (i + 1) * FH)
            if i == 1:
                ln(TB + u * 128)
        w1u_ref[:, i * FH:(i + 1) * FH] = pltpu.bitcast(w1_ref[:, i * FH:(i + 1) * FH], U32)

    def pro_body(b, c):
        @pl.when(b + 1 < NB)
        def _():
            cp_x(b + 1).wait()
            wait_group(b - 1)
        z = lax.shift_right_logical(b, 10)
        pro_block(b, True, b - 1, z.astype(U32))
        return z
    z_last = lax.fori_loop(1, NB - 1, pro_body, jnp.int32(0))

    @pl.when(z_last == 0)
    def _():
        wait_group(NG - 1)
        cp_w2.wait()
    pro_block(NB - 1, False, NG - 1, z_last.astype(U32), extra=list(range(F // 128)))

    def store_next(Rh, h, r0):
        hs = slice(h * 256, (h + 1) * 256)
        q8a_ref[:, hs] = Rh[r0:r0 + 8, 0:256]
        q16_ref[:, hs] = Rh[r0 + 8:r0 + 24, 0:256].astype(BF)
        q8b_ref[:, hs] = Rh[r0 + 24:r0 + 32, 0:256]
        kg_ref[:, hs] = Rh[r0:r0 + 32, 256:512].astype(BF)
        vg_ref[:, hs] = Rh[r0:r0 + 32, 512:768].astype(BF)

    def wcols(h, z):
        return _bf(w_ref, (pl.ds(z, D // 2), slice(h * 768, (h + 1) * 768)))

    lhs0 = xn_ref[0:32, :].astype(BF)
    WO = lambda a, b: [lambda h=h: wo_unit(h) for h in range(a, b)]
    plan = [([cp_wo(0), cp_wo(1)], range(0, 8), WO(0, 8)),
            ([cp_wo(2)], range(8, 12), WO(8, 12)),
            ([cp_wo(3), cp_m], range(12, 16), WO(12, 16))]
    for waits, heads, side in plan:
        @pl.when(z_last == 0)
        def _():
            for c in waits:
                c.wait()
        done = 0
        for n, h in enumerate(heads):
            store_next(jnp.dot(lhs0, wcols(h, 0), preferred_element_type=F32), h, 0)
            upto = (n + 1) * len(side) // len(heads)
            for fn in side[done:upto]:
                fn()
            done = upto

    def out_block(t0, z=None):
        cols = _ds(t0, 128, 128)
        y = xT_ref[:, cols].astype(F32) + orow_ref[cols, :].T
        outT_ref[:, cols] = y.astype(BF)
        if z is None:
            return None
        bits = pltpu.bitcast(y, U32)
        acc = bits[0:8]
        for r in range(8, D, 8):
            acc = acc | bits[r:r + 8]
        return acc & jnp.full((8, 128), z, U32)

    def pin(mem, dep):
        head = pltpu.bitcast(pltpu.bitcast(mem[:, 0:128], U32) | dep, F32)
        return jnp.concatenate([head, mem[:, 128:]], axis=1)

    def cp_out(t0):
        cols = _ds(t0, 128, 128)
        return pltpu.make_async_copy(outT_ref.at[:, cols], outT_hbm.at[:, cols], osem)

    def pair(p, mem, sub, last=False):
        if isinstance(p, int):
            base, nxt, zsrc, zsh = p * 64, p * 64 + 64, z_last, 1
        else:
            base = pl.multiple_of(p * 64, 64)
            nxt, zsrc, zsh = pl.multiple_of(base + 64, 64), p, 10
        z = [pl.multiple_of(lax.shift_right_logical(zsrc, zsh + i + 2 * sub) * 8, 8) for i in range(2)]
        cap = (ce_ref[...], co_ref[...])
        FF = []

        def ffn2(j0, j1):
            a = act_ref[pl.ds(base, 64), j0 * 128:j1 * 128]
            FF.append(jnp.dot(a, _bf(w2u_ref, (slice(j0 * 64, j1 * 64), slice(None))),
                              preferred_element_type=F32))

        def out_proj(o, e):
            return jnp.dot(jnp.concatenate(o, axis=1), _bf(wo_ref, (pl.ds(z[e], H * DH // 2), slice(None))),
                           preferred_element_type=F32)

        lhs = jnp.concatenate([mem, xn_ref[pl.ds(base + 32, 24), :]], axis=0).astype(BF)
        R = [jnp.dot(lhs, wcols(h, z[0]), preferred_element_type=F32) for h in range(H)]
        keep, sc = [], []
        for h in range(H):
            hs = slice(h * 256, (h + 1) * 256)
            gb = R[h][16:32, :].astype(BF)
            gkv = R[h][0:16, 256:768].astype(BF)
            q = jnp.concatenate([
                jnp.concatenate([R[h][0:8, 0:256], q8a_ref[:, hs]], axis=0).astype(BF),
                q16_ref[:, hs]], axis=0)
            k = jnp.concatenate([kg_ref[:, hs], gkv[:, 0:256]], axis=0)
            keep.append((R[h][8:16, 0:256], gkv, gb))
            sc.append(lax.dot_general(q, k, NT, preferred_element_type=F32))
        ffn2(0, 4)
        o = []
        for h in range(H):
            v = jnp.concatenate([vg_ref[:, h * 256:(h + 1) * 256], keep[h][1][:, 256:512]], axis=0)
            o.append(jnp.dot(_softmax_p(sc[h], cap[0]), v, preferred_element_type=F32).astype(BF))
        Ce = out_proj(o, 0)
        ffn2(4, 7)

        parts = [Ce[0:8], xn_ref[pl.ds(base + 56, 8), :]]
        if not last:
            parts.append(xn_ref[pl.ds(nxt, 32), :])
        lhs = jnp.concatenate(parts, axis=0).astype(BF)
        R = [jnp.dot(lhs, wcols(h, z[1]), preferred_element_type=F32) for h in range(H)]
        gcs, sc = [], []
        for h in range(H):
            hs = slice(h * 256, (h + 1) * 256)
            qa, gkv, gb = keep[h]
            gc = R[h][0:16, :].astype(BF)
            q = jnp.concatenate([
                gc[:, 0:256], gb[:, 0:256],
                jnp.concatenate([q8b_ref[:, hs], qa], axis=0).astype(BF)], axis=0)
            k = jnp.concatenate([kg_ref[:, hs], gkv[:, 0:256], gb[:, 256:512], gc[:, 256:512]], axis=0)
            gcs.append(gc)
            sc.append(lax.dot_general(q, k, NT, preferred_element_type=F32))
        ffn2(7, 11)
        o = []
        for h in range(H):
            _, gkv, gb = keep[h]
            v = jnp.concatenate([vg_ref[:, h * 256:(h + 1) * 256], gkv[:, 256:512], gb[:, 512:768],
                                 gcs[h][:, 512:768]], axis=0)
            o.append(jnp.dot(_softmax_p(sc[h], cap[1]), v, preferred_element_type=F32).astype(BF))
        Co = out_proj(o, 1)
        if not last:
            for h in range(H):
                store_next(R[h], h, 16)
        ffn2(11, 13)
        ffn2(13, 14)

        tot = jnp.concatenate([Ce[8:32], Co[32:40], Co[40:48], Co[16:32], Co[8:16]], axis=0)
        for f in FF:
            tot = tot + f
        orow_ref[pl.ds(base, 64), :] = tot
        return Co[0:8]

    def body(i, mem):
        if isinstance(i, int):
            tprev = (i - 1) * 128
            out_block(tprev)
            cp_out(tprev).start()
        else:
            tprev = jnp.maximum(i - 1, 0) * 128
            dep = out_block(tprev, lax.shift_right_logical(i, 10).astype(U32))

            @pl.when(i > 0)
            def _():
                cp_out(tprev).start()
        mem = pair(2 * i, mem, 0)
        if not isinstance(i, int):
            mem = pin(mem, dep)
        return pair(2 * i + 1, mem, 1, last=isinstance(i, int))
    mem = lax.fori_loop(0, NPAIR // 2 - 1, body, mem0_ref[...].astype(F32))
    body(NPAIR // 2 - 1, mem)

    out_block(S - 128)
    cp_out(S - 128).start()
    for b in range(S // 128):
        cp_out(b * 128).wait()


@jax.jit
def pallas_parallel_sum__memory_aug_recurrent_mem_tr__dense_activation_silu__prompt_kernel(
    A_x, A_mem0, A_Wq, A_Wk, A_Wv, A_Wo, A_seg_len, B_x, B_w1, B_w2,
):
    hbm = pl.BlockSpec(memory_space=pltpu.HBM)
    outT = pl.pallas_call(
        _kernel,
        out_shape=jax.ShapeDtypeStruct((D, S), BF),
        in_specs=[hbm] * 8,
        out_specs=hbm,
        scratch_shapes=[
            pltpu.VMEM((D, S), BF),
            pltpu.VMEM((M, D), BF),
            pltpu.VMEM((6, D * H, 128), BF),
            pltpu.VMEM((H, D, DH), BF),
            pltpu.VMEM((D, F), BF),
            pltpu.VMEM((D, F), BF),
            pltpu.VMEM((D, S), BF),
            pltpu.VMEM((S, D), F32),
            pltpu.VMEM((S // 2, D), U32),
            pltpu.VMEM((D // 2, 3 * H * DH), U32),
            pltpu.VMEM((H * DH // 2, D), U32),
            pltpu.VMEM((D // 2, F), U32),
            pltpu.VMEM((F // 2, D), U32),
            pltpu.VMEM((S, D), F32),
            pltpu.VMEM((S, F), BF),
            pltpu.VMEM((32, H * DH), BF),
            pltpu.VMEM((32, H * DH), BF),
            pltpu.VMEM((8, H * DH), F32),
            pltpu.VMEM((16, H * DH), BF),
            pltpu.VMEM((8, H * DH), F32),
            pltpu.VMEM((32, 48), F32),
            pltpu.VMEM((48, 80), F32),
            pltpu.SemaphoreType.DMA((8,)),
            pltpu.SemaphoreType.DMA((NB,)),
            pltpu.SemaphoreType.DMA((NG,)),
            pltpu.SemaphoreType.DMA(()),
        ],
        compiler_params=pltpu.CompilerParams(vmem_limit_bytes=110 * 1024 * 1024),
    )(jnp.swapaxes(A_x, 1, 2).reshape(D, S), A_mem0.reshape(M, D),
      A_Wq.reshape(D * H, DH), A_Wk.reshape(D * H, DH), A_Wv.reshape(D * H, DH),
      jnp.swapaxes(A_Wo, 1, 2), B_w1, B_w2.T)
    return jnp.swapaxes(outT.reshape(1, D, S), 1, 2)
```
